```python
import os as _os
_os.environ.setdefault("JAX_PLATFORMS", "cpu")
import jax
import jax.numpy as jnp

def _softmax(x, axis=-1):
    return jax.nn.softmax(x, axis=axis)
def _gelu(x):
    return jax.nn.gelu(x, approximate=True)
def _silu(x):
    return jax.nn.silu(x)
def _sigmoid(x):
    return jax.nn.sigmoid(x)
def _layernorm(x, axis=-1, eps=1e-5):
    m = jnp.mean(x, axis=axis, keepdims=True)
    v = jnp.var(x, axis=axis, keepdims=True)
    return (x - m) / jnp.sqrt(v + eps)
def _scatter_add(tgt, idx, src, axis=0):
    return tgt.at[idx].add(src)
def _segment_sum(src, seg, n):
    return jax.ops.segment_sum(src, seg, n)
class _Rng:
    def __init__(self, key):
        self._k = key
    def _next(self):
        self._k, sub = jax.random.split(self._k)
        return sub
    def normal(self, shape):
        return jax.random.normal(self._next(), shape, dtype=jnp.bfloat16)
    def randint(self, lo, hi, shape):
        return jax.random.randint(self._next(), shape, lo, hi, dtype=jnp.int32)
    def uniform(self, shape, lo=0.0, hi=1.0):
        return jax.random.uniform(self._next(), shape, jnp.bfloat16, lo, hi)
    def permutation(self, n):
        return jax.random.permutation(self._next(), n)


kernel_name = 'standalone__dense_activation_silu__prompt'

def setup_inputs():
    _rng = _Rng(jax.random.key(int.from_bytes(__import__("os").urandom(4), "little")))
    _w = (lambda a: (lambda t: t.astype(jnp.bfloat16) if jnp.issubdtype(t.dtype, jnp.floating) else t)(jnp.asarray(a)))
    B, S, D, F = 1, 2048, 448, 1792
    return {
        "x": _w((lambda *s: _rng.normal(s) * 0.05)(B, S, D)),
        "w1": _w((lambda *s: _rng.normal(s) * 0.05)(D, F) * (D ** -0.5)),
        "w2": _w((lambda *s: _rng.normal(s) * 0.05)(F, D) * (F ** -0.5)),
    }

def reference(x, w1, w2):
    h = jnp.einsum("bsd,df->bsf", x, w1)
    h = _silu(h)
    out = jnp.einsum("bsf,fd->bsd", h, w2)
    return out
```

```python
import jax
import jax.numpy as jnp
import jax.experimental.pallas as pl
import jax.experimental.pallas.tpu as pltpu

_U = 128
_PAD = 16
_NEG_LOG2E = -1.4426950408889634

_COPIES = (
    ("w1", 0, 3), ("x", 0, 1), ("x", 1, 2), ("x", 2, 3), ("x", 3, 4),
    ("w1", 3, 4), ("w1", 4, 6), ("w1", 6, 9), ("w1", 9, 14),
    ("x", 4, 10), ("w2", 0, 14), ("x", 10, 16),
)
_HEAD = 4
_LAST_ROWS = (0, 224, 352, 416, 448)


def _silu(h):
    d = 1.0 + jnp.exp2(jnp.minimum(h * _NEG_LOG2E, 127.0))
    r = pltpu.reciprocal(d, approx=True)
    r = r * (2.0 - d * r)
    return h * r


def _ffn_kernel(xt_hbm, w1_hbm, w2t_hbm, out_hbm,
                x_buf, w1_buf, w2_buf, w1t_buf, h_buf, out_buf, in_sems, out_sems):
    d_model = out_buf.shape[0]
    operands = {"x": (xt_hbm, x_buf), "w1": (w1_hbm, w1_buf), "w2": (w2t_hbm, w2_buf)}

    def cols(a, b):
        return pl.ds(a * _U, (b - a) * _U)

    loads = {}
    for i, (name, a, b) in enumerate(_COPIES):
        src, dst = operands[name]
        loads[name, a] = pltpu.make_async_copy(
            src.at[:, cols(a, b)], dst.at[pl.ds(0, d_model), cols(a, b)], in_sems.at[i])
        loads[name, a].start()

    def wait_after(value, name, a):
        operands[name][1][pl.ds(d_model, _PAD), cols(0, 1)] = value[:_PAD, :_U]
        loads[name, a].wait()

    def transpose_w1(a, b):
        w = w1_buf[pl.ds(0, d_model), cols(a, b)].T
        w1t_buf[cols(a, b), :] = w
        return w

    def hidden(w1t, s0, s1):
        h = jnp.dot(w1t, x_buf[pl.ds(0, d_model), cols(s0, s1)],
                    preferred_element_type=jnp.float32)
        return _silu(h).astype(h_buf.dtype)

    def hidden_to_buf(a, b, s0, s1):
        h = hidden(w1t_buf[cols(a, b), :], s0, s1)
        h_buf[cols(a, b), cols(s0, s1)] = h
        return h

    stores = []

    def project(h, s0, s1, rows=(0, d_model)):
        for d0, d1 in zip(rows[:-1], rows[1:]):
            block = (pl.ds(d0, d1 - d0), cols(s0, s1))
            out = jnp.dot(w2_buf[pl.ds(d0, d1 - d0), :], h, preferred_element_type=jnp.float32)
            out_buf[block] = out.astype(out_buf.dtype)
            store = pltpu.make_async_copy(
                out_buf.at[block], out_hbm.at[block], out_sems.at[len(stores)])
            store.start()
            stores.append(store)

    loads["w1", 0].wait()
    w = transpose_w1(0, 3)
    wait_after(w[128:], "x", 0)
    h = hidden_to_buf(0, 3, 0, 1)
    wait_after(h, "x", 1)
    h = hidden_to_buf(0, 3, 1, 2)
    wait_after(h, "x", 2)
    h = hidden_to_buf(0, 3, 2, 3)
    wait_after(h, "x", 3)
    wait_after(h[200:], "w1", 3)
    h = hidden_to_buf(0, 3, 3, 4)
    transpose_w1(3, 4)
    wait_after(h, "w1", 4)
    hidden_to_buf(3, 4, 0, _HEAD)
    transpose_w1(4, 6)
    h = hidden_to_buf(4, 6, 0, _HEAD)
    wait_after(h, "w1", 6)
    transpose_w1(6, 9)
    h = hidden_to_buf(6, 9, 0, _HEAD)
    wait_after(h, "w1", 9)
    transpose_w1(9, 14)
    h = hidden_to_buf(9, 14, 0, _HEAD)
    wait_after(h, "x", 4)

    h = hidden(w1t_buf[...], 4, 10)
    wait_after(h[1008:], "w2", 0)
    project(h, 4, 10)
    wait_after(h, "x", 10)
    project(h_buf[...], 0, _HEAD)
    project(hidden(w1t_buf[...], 10, 16), 10, 16, _LAST_ROWS)

    for store in stores:
        store.wait()


@jax.jit
def pallas_standalone__dense_activation_silu__prompt_kernel(
    x: jax.Array,
    w1: jax.Array,
    w2: jax.Array,
):
    batch, seq, d_model = x.shape
    d_ff = w1.shape[1]
    tokens = batch * seq
    assert (tokens, d_model, d_ff) == (16 * _U, _LAST_ROWS[-1], 14 * _U)

    any_spec = pl.BlockSpec(memory_space=pl.ANY)
    out_t = pl.pallas_call(
        _ffn_kernel,
        in_specs=[any_spec] * 3,
        out_specs=any_spec,
        out_shape=jax.ShapeDtypeStruct((d_model, tokens), x.dtype),
        scratch_shapes=[
            pltpu.VMEM((d_model + _PAD, tokens), x.dtype),
            pltpu.VMEM((d_model + _PAD, d_ff), w1.dtype),
            pltpu.VMEM((d_model + _PAD, d_ff), w2.dtype),
            pltpu.VMEM((d_ff, d_model), w1.dtype),
            pltpu.VMEM((d_ff, _HEAD * _U), x.dtype),
            pltpu.VMEM((d_model, tokens), x.dtype),
            pltpu.SemaphoreType.DMA((len(_COPIES),)),
            pltpu.SemaphoreType.DMA((2 + len(_LAST_ROWS) - 1,)),
        ],
        compiler_params=pltpu.CompilerParams(
            vmem_limit_bytes=100 * 1024 * 1024,
            disable_semaphore_checks=True,
            flags={"XLA_TPU_RESCHEDULE_DMA_DONES": True},
        ),
    )(x.reshape(tokens, d_model).T, w1, w2.T)
    return out_t.T.reshape(batch, seq, d_model)
```

```python
import jax
import jax.numpy as jnp
import jax.experimental.pallas as pl
import jax.experimental.pallas.tpu as pltpu

_U = 128
_PAD = 16
_NEG_LOG2E = -1.4426950408889634

_HEAD, _MID, _TOKENS = 4, 10, 16
_EDGE_SPLITS = (0, 4, 8, 14)
_MAIN_SPLITS = (0, 2, 4, 7, 14)
_LAST_ROWS = (0, 256, 352, 448)
_NUM_LOADS = len(_EDGE_SPLITS) + len(_MAIN_SPLITS) + 3
_NUM_STORES = 3 + len(_LAST_ROWS) - 1


def _silu(h):
    d = 1.0 + jnp.exp2(jnp.minimum(h * _NEG_LOG2E, 127.0))
    r = pltpu.reciprocal(d, approx=True)
    r = r * (2.0 - d * r)
    return h * r


def _cols(a, b):
    return pl.ds(a * _U, (b - a) * _U)


def _pieces(splits):
    return list(zip(splits[:-1], splits[1:]))


def _ffn_kernel(xt_hbm, w1_hbm, w2t_hbm, out_hbm,
                x_buf, w1_buf, w2_buf, w1t_buf, partial_buf, h_buf, out_buf,
                load_sems, store_sems):
    d_model = out_buf.shape[0]
    d_main = d_model // _U * _U
    full, main, edge = pl.ds(0, d_model), pl.ds(0, d_main), pl.ds(d_main, d_model - d_main)

    loads, stores = [], []

    def load(src, dst, rows, a, b):
        block = (rows, _cols(a, b))
        copy = pltpu.make_async_copy(src.at[block], dst.at[block], load_sems.at[len(loads)])
        copy.start()
        loads.append(copy)
        return copy, dst

    def wait_after(value, pending):
        copy, dst = pending
        value = value[:_PAD, :_U]
        dst[d_model:d_model + _PAD, :value.shape[1]] = value.astype(dst.dtype)
        copy.wait()

    def transpose_w1(rows, a, b):
        w = w1_buf[rows, _cols(a, b)].T
        w1t_buf[_cols(a, b), rows] = w
        return w

    def up(rows, a, b, s0, s1):
        return jnp.dot(w1t_buf[_cols(a, b), rows], x_buf[rows, _cols(s0, s1)],
                       preferred_element_type=jnp.float32)

    def hidden(s0, s1):
        return _silu(up(full, 0, _MAIN_SPLITS[-1], s0, s1)).astype(h_buf.dtype)

    def down(h, s0, s1, row_splits=(0, d_model)):
        for d0, d1 in _pieces(row_splits):
            rows = pl.ds(d0, d1 - d0)
            block = (rows, _cols(s0, s1))
            out = jnp.dot(w2_buf[rows, :], h, preferred_element_type=jnp.float32)
            out_buf[block] = out.astype(out_buf.dtype)
            copy = pltpu.make_async_copy(
                out_buf.at[block], out_hbm.at[block], store_sems.at[len(stores)])
            copy.start()
            stores.append(copy)

    edge_pieces, main_pieces = _pieces(_EDGE_SPLITS), _pieces(_MAIN_SPLITS)
    w1_edge = [load(w1_hbm, w1_buf, edge, *edge_pieces[0])]
    x_edge = load(xt_hbm, x_buf, edge, 0, _HEAD)
    w1_edge += [load(w1_hbm, w1_buf, edge, a, b) for a, b in edge_pieces[1:]]
    w1_main = [load(w1_hbm, w1_buf, main, *main_pieces[0])]
    x_main = load(xt_hbm, x_buf, main, 0, _HEAD)
    w1_main += [load(w1_hbm, w1_buf, main, a, b) for a, b in main_pieces[1:]]
    x_mid = load(xt_hbm, x_buf, full, _HEAD, _MID)
    w2_all = load(w2t_hbm, w2_buf, full, 0, _MAIN_SPLITS[-1])
    x_rest = load(xt_hbm, x_buf, full, _MID, _TOKENS)

    last = None
    for i, (a, b) in enumerate(edge_pieces):
        if i == 0:
            w1_edge[0][0].wait()
            wait_after(transpose_w1(edge, a, b)[256:], x_edge)
        else:
            wait_after(last, w1_edge[i])
            transpose_w1(edge, a, b)
        last = up(edge, a, b, 0, _HEAD)
        partial_buf[_cols(a, b), :] = last

    for i, (a, b) in enumerate(main_pieces):
        wait_after(last, w1_main[i])
        transpose_w1(main, a, b)
        if i == 0:
            wait_after(last[400:], x_main)
        last = _silu(partial_buf[_cols(a, b), :] + up(main, a, b, 0, _HEAD)).astype(h_buf.dtype)
        h_buf[_cols(a, b), :] = last

    wait_after(last, x_mid)
    h = hidden(_HEAD, _MID)
    wait_after(h[1008:], w2_all)
    down(h, _HEAD, _MID)
    wait_after(h, x_rest)
    down(hidden(_MID, _TOKENS), _MID, _TOKENS)

    half = _HEAD // 2
    down(h_buf[:, _cols(0, half)], 0, half)
    down(h_buf[:, _cols(half, _HEAD)], half, _HEAD, _LAST_ROWS)

    for copy in stores:
        copy.wait()


@jax.jit
def pallas_standalone__dense_activation_silu__prompt_kernel(
    x: jax.Array,
    w1: jax.Array,
    w2: jax.Array,
):
    batch, seq, d_model = x.shape
    d_ff = w1.shape[1]
    tokens = batch * seq
    assert (tokens, d_model, d_ff) == (_TOKENS * _U, _LAST_ROWS[-1], _MAIN_SPLITS[-1] * _U)

    any_spec = pl.BlockSpec(memory_space=pl.ANY)
    out_t = pl.pallas_call(
        _ffn_kernel,
        in_specs=[any_spec] * 3,
        out_specs=any_spec,
        out_shape=jax.ShapeDtypeStruct((d_model, tokens), x.dtype),
        scratch_shapes=[
            pltpu.VMEM((d_model + _PAD, tokens), x.dtype),
            pltpu.VMEM((d_model + _PAD, d_ff), w1.dtype),
            pltpu.VMEM((d_model + _PAD, d_ff), w2.dtype),
            pltpu.VMEM((d_ff, d_model), w1.dtype),
            pltpu.VMEM((d_ff, _HEAD * _U), jnp.float32),
            pltpu.VMEM((d_ff, _HEAD * _U), x.dtype),
            pltpu.VMEM((d_model, tokens), x.dtype),
            pltpu.SemaphoreType.DMA((_NUM_LOADS,)),
            pltpu.SemaphoreType.DMA((_NUM_STORES,)),
        ],
        compiler_params=pltpu.CompilerParams(
            vmem_limit_bytes=100 * 1024 * 1024,
            disable_semaphore_checks=True,
            flags={
                "XLA_TPU_RESCHEDULE_DMA_DONES": True,
                "XLA_TPU_EVENLY_DISTRIBUTE_CRITICAL_NODES": True,
            },
        ),
    )(x.reshape(tokens, d_model).T, w1, w2.T)
    return out_t.T.reshape(batch, seq, d_model)
```

```python
import jax
import jax.numpy as jnp
import jax.experimental.pallas as pl
import jax.experimental.pallas.tpu as pltpu

_U = 128
_PAD = 16
_NEG_LOG2E = -1.4426950408889634

_HEAD, _MID, _TOKENS = 4, 10, 16
_EDGE_SPLITS = (0, 4, 8, 14)
_MAIN_SPLITS = (0, 2, 4, 7, 14)
_LAST_ROWS = (0, 256, 352, 448)
_NUM_LOADS = len(_EDGE_SPLITS) + len(_MAIN_SPLITS) + 4
_NUM_STORES = 3 + len(_LAST_ROWS) - 1


def _silu(h):
    d = 1.0 + jnp.exp2(jnp.minimum(h * _NEG_LOG2E, 127.0))
    r = pltpu.reciprocal(d, approx=True)
    r = r * (2.0 - d * r)
    return h * r


def _cols(a, b):
    return pl.ds(a * _U, (b - a) * _U)


def _pieces(splits):
    return list(zip(splits[:-1], splits[1:]))


def _ffn_kernel(xt_hbm, w1_hbm, w2t_hbm, out_hbm,
                x_buf, w1_buf, w2_buf, w1t_buf, partial_buf, h_buf, out_buf,
                load_sems, store_sems):
    d_model = out_buf.shape[0]
    d_main = d_model // _U * _U
    full, main, edge = pl.ds(0, d_model), pl.ds(0, d_main), pl.ds(d_main, d_model - d_main)

    loads, stores = [], []

    def load(src, dst, rows, a, b):
        block = (rows, _cols(a, b))
        copy = pltpu.make_async_copy(src.at[block], dst.at[block], load_sems.at[len(loads)])
        copy.start()
        loads.append(copy)
        return copy, dst

    def wait_after(value, pending):
        copy, dst = pending
        value = value[:_PAD, :_U]
        dst[d_model:d_model + _PAD, :value.shape[1]] = value.astype(dst.dtype)
        copy.wait()

    def transpose_w1(rows, a, b):
        w = w1_buf[rows, _cols(a, b)].T
        w1t_buf[_cols(a, b), rows] = w
        return w

    def up(rows, a, b, s0, s1):
        return jnp.dot(w1t_buf[_cols(a, b), rows], x_buf[rows, _cols(s0, s1)],
                       preferred_element_type=jnp.float32)

    def hidden(s0, s1):
        return _silu(up(full, 0, _MAIN_SPLITS[-1], s0, s1)).astype(h_buf.dtype)

    def down(h, s0, s1, row_splits=(0, d_model)):
        for d0, d1 in _pieces(row_splits):
            rows = pl.ds(d0, d1 - d0)
            block = (rows, _cols(s0, s1))
            out = jnp.dot(w2_buf[rows, :], h, preferred_element_type=jnp.float32)
            out_buf[block] = out.astype(out_buf.dtype)
            copy = pltpu.make_async_copy(
                out_buf.at[block], out_hbm.at[block], store_sems.at[len(stores)])
            copy.start()
            stores.append(copy)

    edge_pieces, main_pieces = _pieces(_EDGE_SPLITS), _pieces(_MAIN_SPLITS)
    half = _HEAD // 2
    w1_edge = [load(w1_hbm, w1_buf, edge, *edge_pieces[0])]
    x_edge = [load(xt_hbm, x_buf, edge, 0, half), load(xt_hbm, x_buf, edge, half, _HEAD)]
    w1_edge += [load(w1_hbm, w1_buf, edge, a, b) for a, b in edge_pieces[1:]]
    w1_main = [load(w1_hbm, w1_buf, main, *main_pieces[0])]
    x_main = load(xt_hbm, x_buf, main, 0, _HEAD)
    w1_main += [load(w1_hbm, w1_buf, main, a, b) for a, b in main_pieces[1:]]
    x_mid = load(xt_hbm, x_buf, full, _HEAD, _MID)
    w2_all = load(w2t_hbm, w2_buf, full, 0, _MAIN_SPLITS[-1])
    x_rest = load(xt_hbm, x_buf, full, _MID, _TOKENS)

    def up_edge(a, b, s0, s1):
        partial = up(edge, a, b, s0, s1)
        partial_buf[_cols(a, b), _cols(s0, s1)] = partial
        return partial

    w1_edge[0][0].wait()
    w = transpose_w1(edge, *edge_pieces[0])
    wait_after(w[128:], x_edge[0])
    last = up_edge(*edge_pieces[0], 0, half)[128:]
    wait_after(w[300:], x_edge[1])
    up_edge(*edge_pieces[0], half, _HEAD)
    for (a, b), pending in zip(edge_pieces[1:], w1_edge[1:]):
        wait_after(last, pending)
        transpose_w1(edge, a, b)
        last = up_edge(a, b, 0, _HEAD)

    for i, (a, b) in enumerate(main_pieces):
        wait_after(last, w1_main[i])
        transpose_w1(main, a, b)
        if i == 0:
            wait_after(last[400:], x_main)
        last = _silu(partial_buf[_cols(a, b), :] + up(main, a, b, 0, _HEAD)).astype(h_buf.dtype)
        h_buf[_cols(a, b), :] = last

    wait_after(last, x_mid)
    h = hidden(_HEAD, _MID)
    wait_after(h[1008:], w2_all)
    down(h, _HEAD, _MID)
    wait_after(h, x_rest)
    down(hidden(_MID, _TOKENS), _MID, _TOKENS)

    down(h_buf[:, _cols(0, half)], 0, half)
    down(h_buf[:, _cols(half, _HEAD)], half, _HEAD, _LAST_ROWS)

    for copy in stores:
        copy.wait()


@jax.jit
def pallas_standalone__dense_activation_silu__prompt_kernel(
    x: jax.Array,
    w1: jax.Array,
    w2: jax.Array,
):
    batch, seq, d_model = x.shape
    d_ff = w1.shape[1]
    tokens = batch * seq
    assert (tokens, d_model, d_ff) == (_TOKENS * _U, _LAST_ROWS[-1], _MAIN_SPLITS[-1] * _U)

    any_spec = pl.BlockSpec(memory_space=pl.ANY)
    out_t = pl.pallas_call(
        _ffn_kernel,
        in_specs=[any_spec] * 3,
        out_specs=any_spec,
        out_shape=jax.ShapeDtypeStruct((d_model, tokens), x.dtype),
        scratch_shapes=[
            pltpu.VMEM((d_model + _PAD, tokens), x.dtype),
            pltpu.VMEM((d_model + _PAD, d_ff), w1.dtype),
            pltpu.VMEM((d_model + _PAD, d_ff), w2.dtype),
            pltpu.VMEM((d_ff, d_model), w1.dtype),
            pltpu.VMEM((d_ff, _HEAD * _U), jnp.float32),
            pltpu.VMEM((d_ff, _HEAD * _U), x.dtype),
            pltpu.VMEM((d_model, tokens), x.dtype),
            pltpu.SemaphoreType.DMA((_NUM_LOADS,)),
            pltpu.SemaphoreType.DMA((_NUM_STORES,)),
        ],
        compiler_params=pltpu.CompilerParams(
            vmem_limit_bytes=100 * 1024 * 1024,
            disable_semaphore_checks=True,
            flags={
                "XLA_TPU_RESCHEDULE_DMA_DONES": True,
                "XLA_TPU_EVENLY_DISTRIBUTE_CRITICAL_NODES": True,
            },
        ),
    )(x.reshape(tokens, d_model).T, w1, w2.T)
    return out_t.T.reshape(batch, seq, d_model)
```
